```python
import os as _os
_os.environ.setdefault("JAX_PLATFORMS", "cpu")
import jax
import jax.numpy as jnp

def _softmax(x, axis=-1):
    return jax.nn.softmax(x, axis=axis)
def _gelu(x):
    return jax.nn.gelu(x, approximate=True)
def _silu(x):
    return jax.nn.silu(x)
def _sigmoid(x):
    return jax.nn.sigmoid(x)
def _layernorm(x, axis=-1, eps=1e-5):
    m = jnp.mean(x, axis=axis, keepdims=True)
    v = jnp.var(x, axis=axis, keepdims=True)
    return (x - m) / jnp.sqrt(v + eps)
def _scatter_add(tgt, idx, src, axis=0):
    return tgt.at[idx].add(src)
def _segment_sum(src, seg, n):
    return jax.ops.segment_sum(src, seg, n)
class _Rng:
    def __init__(self, key):
        self._k = key
    def _next(self):
        self._k, sub = jax.random.split(self._k)
        return sub
    def normal(self, shape):
        return jax.random.normal(self._next(), shape, dtype=jnp.bfloat16)
    def randint(self, lo, hi, shape):
        return jax.random.randint(self._next(), shape, lo, hi, dtype=jnp.int32)
    def uniform(self, shape, lo=0.0, hi=1.0):
        return jax.random.uniform(self._next(), shape, jnp.bfloat16, lo, hi)
    def permutation(self, n):
        return jax.random.permutation(self._next(), n)


kernel_name = 'standalone__dense_activation_gelu__prompt'

def setup_inputs():
    _rng = _Rng(jax.random.key(int.from_bytes(__import__("os").urandom(4), "little")))
    _w = (lambda a: (lambda t: t.astype(jnp.bfloat16) if jnp.issubdtype(t.dtype, jnp.floating) else t)(jnp.asarray(a)))
    B, S, D, F = 1, 2048, 640, 1728
    return {
        "x": _w((lambda *s: _rng.normal(s) * 0.05)(B, S, D)),
        "w1": _w((lambda *s: _rng.normal(s) * 0.05)(D, F) * (D ** -0.5)),
        "b1": _w((lambda *s: _rng.normal(s) * 0.05)(F) * 0.01),
        "w2": _w((lambda *s: _rng.normal(s) * 0.05)(F, D) * (F ** -0.5)),
        "b2": _w((lambda *s: _rng.normal(s) * 0.05)(D) * 0.01),
    }

def reference(x, w1, b1, w2, b2):
    h = jnp.einsum("bsd,df->bsf", x, w1) + b1
    h = _gelu(h)
    return jnp.einsum("bsf,fd->bsd", h, w2) + b2
```

```python
import jax
import jax.experimental.pallas as pl
import jax.experimental.pallas.tpu as pltpu
import jax.numpy as jnp
import numpy as np
from jax import lax

_NT = (((1,), (1,)), ((), ()))


def _gelu(h):
    c = np.float32(np.sqrt(2.0 / np.pi))
    inner = c * (h + np.float32(0.044715) * (h * h * h))
    return np.float32(0.5) * h * (np.float32(1.0) + jnp.tanh(inner))


@jax.jit
def pallas_standalone__dense_activation_gelu__prompt_kernel(
    x: jax.Array,
    w1: jax.Array,
    b1: jax.Array,
    w2: jax.Array,
    b2: jax.Array,
):
    B, S0, D = x.shape
    S = B * S0
    F = w1.shape[1]

    tm = 512
    assert S % tm == 0 and S // tm >= 2
    nb = S // tm
    gs = [(0, 256), (256, 512), (768, 512), (1280, F - 1280)]
    ng = len(gs)
    pieces = [(0, tm, 0, 512), (0, 384, 512, D - 512), (384, tm - 384, 512, D - 512)]
    SX0, SB1, SW1, SW2, SB2, SXR, SO = 0, 1, 2, 2 + ng, 3 + ng, 4 + ng, 5 + ng
    nsem = SO + (nb - 1) + len(pieces)

    def kern(x_hbm, w1t_hbm, b1_hbm, w2_hbm, b2_hbm, o_hbm,
             xb, w1b, w2b, b1b, b2b, ob, hb, sem):
        mk = pltpu.make_async_copy
        cx0 = mk(x_hbm.at[pl.ds(0, tm)], xb.at[pl.ds(0, tm)], sem.at[SX0])
        cxr = mk(x_hbm.at[pl.ds(tm, S - tm)], xb.at[pl.ds(tm, S - tm)], sem.at[SXR])
        cb1 = mk(b1_hbm, b1b, sem.at[SB1])
        cb2 = mk(b2_hbm, b2b, sem.at[SB2])
        cw1 = [mk(w1t_hbm.at[pl.ds(a, n)], w1b.at[pl.ds(a, n)], sem.at[SW1 + j])
               for j, (a, n) in enumerate(gs)]
        cw2 = mk(w2_hbm, w2b, sem.at[SW2])
        cb1.start()
        cw1[0].start()
        cx0.start()
        for j in range(1, ng):
            cw1[j].start()
        cw2.start()
        cb2.start()
        cxr.start()
        outs = []
        for i in range(nb):
            if i == 0:
                cb1.wait()
                cw1[0].wait()
                cx0.wait()
                for j, (a, n) in enumerate(gs):
                    if j > 0:
                        cw1[j].wait()
                    raw = lax.dot_general(xb[pl.ds(0, tm), :], w1b[pl.ds(a, n), :], _NT,
                                          preferred_element_type=jnp.float32)
                    b = b1b[pl.ds(a, n)].astype(jnp.float32).reshape(1, n)
                    hb[:, pl.ds(a, n)] = _gelu(raw + b).astype(jnp.bfloat16)
                cw2.wait()
                cb2.wait()
                h = hb[...]
            else:
                if i == 1:
                    cxr.wait()
                h = lax.dot_general(xb[pl.ds(i * tm, tm), :], w1b[...], _NT,
                                    preferred_element_type=jnp.float32)
                b1v = b1b[...].astype(jnp.float32).reshape(1, F)
                h = _gelu(h + b1v).astype(jnp.bfloat16)
            if i < nb - 1:
                acc = jnp.dot(h, w2b[...], preferred_element_type=jnp.float32)
                b2v = b2b[...].astype(jnp.float32).reshape(1, D)
                ob[pl.ds(i * tm, tm), :] = (acc + b2v).astype(jnp.bfloat16)
                c = mk(ob.at[pl.ds(i * tm, tm)], o_hbm.at[pl.ds(i * tm, tm)], sem.at[SO + len(outs)])
                c.start()
                outs.append(c)
            else:
                for (pr, pn, pc, pcn) in pieces:
                    hh = h if pn == tm else h[pr:pr + pn]
                    acc = jnp.dot(hh, w2b[:, pl.ds(pc, pcn)], preferred_element_type=jnp.float32)
                    b2v = b2b[pl.ds(pc, pcn)].astype(jnp.float32).reshape(1, pcn)
                    r = i * tm + pr
                    ob[pl.ds(r, pn), pl.ds(pc, pcn)] = (acc + b2v).astype(jnp.bfloat16)
                    c = mk(ob.at[pl.ds(r, pn), pl.ds(pc, pcn)],
                           o_hbm.at[pl.ds(r, pn), pl.ds(pc, pcn)], sem.at[SO + len(outs)])
                    c.start()
                    outs.append(c)
        for c in outs:
            c.wait()

    any_ = pl.BlockSpec(memory_space=pl.ANY)
    out = pl.pallas_call(
        kern,
        in_specs=[any_] * 5,
        out_specs=any_,
        out_shape=jax.ShapeDtypeStruct((S, D), x.dtype),
        scratch_shapes=[
            pltpu.VMEM((S, D), jnp.bfloat16),
            pltpu.VMEM((F, D), jnp.bfloat16),
            pltpu.VMEM((F, D), jnp.bfloat16),
            pltpu.VMEM((F,), jnp.bfloat16),
            pltpu.VMEM((D,), jnp.bfloat16),
            pltpu.VMEM((S, D), jnp.bfloat16),
            pltpu.VMEM((tm, F), jnp.bfloat16),
            pltpu.SemaphoreType.DMA((nsem,)),
        ],
        compiler_params=pltpu.CompilerParams(vmem_limit_bytes=96 * 1024 * 1024),
    )(x.reshape(S, D), w1.T, b1, w2, b2)
    return out.reshape(B, S0, D)
```

```python
import jax
import jax.experimental.pallas as pl
import jax.experimental.pallas.tpu as pltpu
import jax.numpy as jnp
import numpy as np
from jax import lax

_F32 = jnp.float32
_BF16 = jnp.bfloat16
_LANE = 128
_NT = (((1,), (1,)), ((), ()))


def _gelu(h):
    c = np.float32(np.sqrt(2.0 / np.pi))
    inner = c * (h + np.float32(0.044715) * (h * h * h))
    return np.float32(0.5) * h * (np.float32(1.0) + jnp.tanh(inner))


def _dot_nt(a, b):
    return lax.dot_general(a, b, _NT, preferred_element_type=_F32)


def _dot_nn(a, b):
    return jnp.dot(a, b, preferred_element_type=_F32)


@jax.jit
def pallas_standalone__dense_activation_gelu__prompt_kernel(
    x: jax.Array,
    w1: jax.Array,
    b1: jax.Array,
    w2: jax.Array,
    b2: jax.Array,
):
    B, S0, D = x.shape
    S = B * S0
    F = w1.shape[1]

    FM = (F // _LANE) * _LANE
    FT = F - FM
    FP = FM + _LANE
    KH = 256
    FH1 = 768
    FH2 = FP // 2
    assert FT > 0 and 2 * KH <= D and 2 * FH1 <= FM and FP % (2 * _LANE) == 0
    blocks = (512, 256, 768, 512)
    assert sum(blocks) == S
    roff = [int(v) for v in np.concatenate([[0], np.cumsum(blocks)])]
    r0, r1 = blocks[0], blocks[1]
    R01 = r0 + r1
    groups = [(0, 128), (128, 256), (384, 512), (896, F - 896)]
    gsplit = (4, 2, 1, 1)
    ng = len(groups)
    last_rows = (384, 128)
    assert sum(last_rows) == blocks[-1]
    n_out = (len(blocks) - 2) + 1 + len(last_rows) + 1
    SX0, SB1, SW1, SW2, SB2, SX1, SXR, SO = 0, 1, 2, 2 + ng, 3 + ng, 4 + ng, 5 + ng, 6 + ng
    PC = 32

    def kernel(x_hbm, w1t_hbm, b1_hbm, w2_hbm, b2_hbm, o_hbm,
               xb, w1b, w2b, b1b, b2b, ob, hb, b1c, tb, ub, sem):
        copy = pltpu.make_async_copy
        cx0 = copy(x_hbm.at[pl.ds(0, r0)], xb.at[pl.ds(0, r0)], sem.at[SX0])
        cx1 = copy(x_hbm.at[pl.ds(r0, r1)], xb.at[pl.ds(r0, r1)], sem.at[SX1])
        cxr = copy(x_hbm.at[pl.ds(R01, S - R01)], xb.at[pl.ds(R01, S - R01)], sem.at[SXR])
        cb1 = copy(b1_hbm, b1b, sem.at[SB1])
        cb2 = copy(b2_hbm, b2b, sem.at[SB2])
        cw1 = [copy(w1t_hbm.at[pl.ds(a, n)], w1b.at[pl.ds(a, n)], sem.at[SW1 + j])
               for j, (a, n) in enumerate(groups)]
        cw2 = copy(w2_hbm, w2b.at[pl.ds(0, F)], sem.at[SW2])

        cb1.start()
        cb2.start()
        cw1[0].start()
        cx0.start()
        for j in range(1, ng):
            cw1[j].start()
        cx1.start()
        cw2.start()
        cxr.start()
        w2b[pl.ds(F, FP - F), :] = jnp.zeros((FP - F, D), _BF16)

        def bias_row(ref, a, n):
            return ref[pl.ds(a, n)].astype(_F32).reshape(1, n)

        def p1_plain(r, n, a, fn):
            raw = _dot_nt(xb[pl.ds(r, n), :], w1b[pl.ds(a, fn), :])
            return _gelu(raw + bias_row(b1b, a, fn))

        def p1_tail(r, n):
            ht = _dot_nt(w1b[pl.ds(FM, FT), :], xb[pl.ds(r, n), :])
            bc = b1c[...]
            if n > _LANE:
                bc = jnp.concatenate([bc] * (n // _LANE), axis=1)
            return _gelu(ht + bc).T

        def p1_strassen(r, n):
            m = n // 2
            ra, rb = r, r + m
            X11 = xb[pl.ds(ra, m), 0:KH]
            X12 = xb[pl.ds(ra, m), KH:2 * KH]
            X21 = xb[pl.ds(rb, m), 0:KH]
            X22 = xb[pl.ds(rb, m), KH:2 * KH]
            a11, a12, a21, a22 = [v.astype(_F32) for v in (X11, X12, X21, X22)]
            S1 = (a11 - a22).astype(_BF16)
            S2 = (a21 - a22).astype(_BF16)
            S5 = (a12 - a11).astype(_BF16)
            S6 = (a21 - a11).astype(_BF16)
            S7 = (a12 - a22).astype(_BF16)
            x3a = xb[pl.ds(ra, m), 2 * KH:D]
            x3b = xb[pl.ds(rb, m), 2 * KH:D]
            q11, q12, q21, q22 = [], [], [], []
            for c0 in range(0, FH1, _LANE):
                ca = pl.ds(c0, _LANE)
                cb = pl.ds(FH1 + c0, _LANE)
                ba = bias_row(b1b, c0, _LANE)
                bb = bias_row(b1b, FH1 + c0, _LANE)
                w31 = w1b[ca, 2 * KH:D]
                w32 = w1b[cb, 2 * KH:D]
                M3 = _dot_nt(X11, tb[1, ca, :])
                M5 = _dot_nt(S5, w1b[cb, KH:2 * KH])
                q12.append(_gelu(M3 + M5 + _dot_nt(x3a, w32) + bb))
                M2 = _dot_nt(S2, w1b[ca, 0:KH])
                M4 = _dot_nt(X22, tb[2, ca, :])
                q21.append(_gelu(M2 + M4 + _dot_nt(x3b, w31) + ba))
                M1 = _dot_nt(S1, tb[0, ca, :])
                M7 = _dot_nt(S7, tb[4, ca, :])
                q11.append(_gelu(M1 + M4 - M5 + M7 + _dot_nt(x3a, w31) + ba))
                M6 = _dot_nt(S6, tb[3, ca, :])
                q22.append(_gelu(M1 - M2 + M3 + M6 + _dot_nt(x3b, w32) + bb))
            top = jnp.concatenate(q11 + q12, axis=1)
            bot = jnp.concatenate(q21 + q22, axis=1)
            return jnp.concatenate([top, bot], axis=0)

        def phase1(r, n):
            return jnp.concatenate(
                [p1_strassen(r, n), p1_plain(r, n, 2 * FH1, FM - 2 * FH1), p1_tail(r, n)], axis=1)

        def combine_w1():
            for a in range(0, FH1, PC):
                d = pl.ds(a, PC)
                e = pl.ds(FH1 + a, PC)
                B11 = w1b[d, 0:KH].astype(_F32)
                B12 = w1b[e, 0:KH].astype(_F32)
                B21 = w1b[d, KH:2 * KH].astype(_F32)
                B22 = w1b[e, KH:2 * KH].astype(_F32)
                tb[0, d, :] = (B11 - B22).astype(_BF16)
                tb[1, d, :] = (B12 + B22).astype(_BF16)
                tb[2, d, :] = (B21 + B11).astype(_BF16)
                tb[3, d, :] = (B11 + B12).astype(_BF16)
                tb[4, d, :] = (B21 + B22).astype(_BF16)

        def combine_w2():
            for a in range(0, FH2, PC):
                d = pl.ds(a, PC)
                e = pl.ds(FH2 + a, PC)
                B11 = w2b[d, 0:KH].astype(_F32)
                B12 = w2b[d, KH:2 * KH].astype(_F32)
                B21 = w2b[e, 0:KH].astype(_F32)
                B22 = w2b[e, KH:2 * KH].astype(_F32)
                ub[0, d, :] = (B11 - B22).astype(_BF16)
                ub[1, d, :] = (B12 + B22).astype(_BF16)
                ub[2, d, :] = (B21 + B11).astype(_BF16)
                ub[3, d, :] = (B11 + B12).astype(_BF16)
                ub[4, d, :] = (B21 + B22).astype(_BF16)

        def p2_plain(G, r, n, c, cn):
            acc = _dot_nn(G.astype(_BF16), w2b[0:F, pl.ds(c, cn)])
            ob[pl.ds(r, n), pl.ds(c, cn)] = (acc + bias_row(b2b, c, cn)).astype(_BF16)

        def p2_strassen(G, r, n):
            m = n // 2
            Gp = jnp.concatenate([G, jnp.zeros((n, FP - F), _F32)], axis=1)
            G11, G12 = Gp[0:m, 0:FH2], Gp[0:m, FH2:FP]
            G21, G22 = Gp[m:n, 0:FH2], Gp[m:n, FH2:FP]
            ca, cb = pl.ds(0, KH), pl.ds(KH, KH)
            ba, bb = bias_row(b2b, 0, KH), bias_row(b2b, KH, KH)
            P5 = _dot_nn((G12 - G11).astype(_BF16), w2b[FH2:FP, cb])
            P3 = _dot_nn(G11.astype(_BF16), ub[1])
            ob[pl.ds(r, m), cb] = (P3 + P5 + bb).astype(_BF16)
            P2 = _dot_nn((G21 - G22).astype(_BF16), w2b[0:FH2, ca])
            P4 = _dot_nn(G22.astype(_BF16), ub[2])
            ob[pl.ds(r + m, m), ca] = (P2 + P4 + ba).astype(_BF16)
            P1 = _dot_nn((G11 - G22).astype(_BF16), ub[0])
            P7 = _dot_nn((G12 - G22).astype(_BF16), ub[4])
            ob[pl.ds(r, m), ca] = (P1 + P4 - P5 + P7 + ba).astype(_BF16)
            P6 = _dot_nn((G21 - G11).astype(_BF16), ub[3])
            ob[pl.ds(r + m, m), cb] = (P1 - P2 + P3 + P6 + bb).astype(_BF16)

        outs = []

        def write_out(r, n, c, cn):
            if cn == D:
                cp = copy(ob.at[pl.ds(r, n)], o_hbm.at[pl.ds(r, n)], sem.at[SO + len(outs)])
            else:
                cp = copy(ob.at[pl.ds(r, n), pl.ds(c, cn)],
                          o_hbm.at[pl.ds(r, n), pl.ds(c, cn)], sem.at[SO + len(outs)])
            cp.start()
            outs.append(cp)

        cb1.wait()
        cw1[0].wait()
        cx0.wait()
        bt = bias_row(b1b, FM, FT)
        b1c[...] = jnp.broadcast_to(bt, (_LANE, FT)).T
        for j, (a, fn) in enumerate(groups):
            if j > 0:
                cw1[j].wait()
            if j == ng - 1:
                cx1.wait()
                combine_w1()
                cb2.wait()
            fm = min(a + fn, FM) - a
            rn = r0 // gsplit[j]
            for s in range(gsplit[j]):
                hb[pl.ds(s * rn, rn), pl.ds(a, fm)] = p1_plain(s * rn, rn, a, fm)
        hb[pl.ds(0, r0), pl.ds(FM, FT)] = p1_tail(0, r0)

        hb[pl.ds(r0, r1), :] = phase1(r0, r1)
        cw2.wait()
        combine_w2()
        cxr.wait()

        G = hb[...]
        p2_strassen(G, 0, R01)
        p2_plain(G, 0, R01, 2 * KH, D - 2 * KH)
        write_out(0, R01, 0, D)

        for i in range(2, len(blocks)):
            r, n = roff[i], blocks[i]
            G = phase1(r, n)
            p2_strassen(G, r, n)
            if i < len(blocks) - 1:
                p2_plain(G, r, n, 2 * KH, D - 2 * KH)
                write_out(r, n, 0, D)
            else:
                write_out(r, n, 0, 2 * KH)
                rr = r
                for rn in last_rows:
                    p2_plain(G[rr - r:rr - r + rn], rr, rn, 2 * KH, D - 2 * KH)
                    write_out(rr, rn, 2 * KH, D - 2 * KH)
                    rr += rn
        for cp in outs:
            cp.wait()

    any_space = pl.BlockSpec(memory_space=pl.ANY)
    out = pl.pallas_call(
        kernel,
        in_specs=[any_space] * 5,
        out_specs=any_space,
        out_shape=jax.ShapeDtypeStruct((S, D), x.dtype),
        scratch_shapes=[
            pltpu.VMEM((S, D), _BF16),
            pltpu.VMEM((F, D), _BF16),
            pltpu.VMEM((FP, D), _BF16),
            pltpu.VMEM((F,), _BF16),
            pltpu.VMEM((D,), _BF16),
            pltpu.VMEM((S, D), _BF16),
            pltpu.VMEM((R01, F), _F32),
            pltpu.VMEM((FT, _LANE), _F32),
            pltpu.VMEM((5, FH1, KH), _BF16),
            pltpu.VMEM((5, FH2, KH), _BF16),
            pltpu.SemaphoreType.DMA((SO + n_out,)),
        ],
        compiler_params=pltpu.CompilerParams(
            vmem_limit_bytes=100 * 1024 * 1024, disable_semaphore_checks=True),
    )(x.reshape(S, D), w1.T, b1, w2, b2)
    return out.reshape(B, S0, D)
```

```python
import jax
import jax.experimental.pallas as pl
import jax.experimental.pallas.tpu as pltpu
import jax.numpy as jnp
import numpy as np
from jax import lax

_F32 = jnp.float32
_BF16 = jnp.bfloat16
_LANE = 128
_NT = (((1,), (1,)), ((), ()))


def _gelu(h):
    c = np.float32(np.sqrt(2.0 / np.pi))
    inner = c * (h + np.float32(0.044715) * (h * h * h))
    return np.float32(0.5) * h * (np.float32(1.0) + jnp.tanh(inner))


def _dot_nt(a, b):
    return lax.dot_general(a, b, _NT, preferred_element_type=_F32)


def _dot_nn(a, b):
    return jnp.dot(a, b, preferred_element_type=_F32)


@jax.jit
def pallas_standalone__dense_activation_gelu__prompt_kernel(
    x: jax.Array,
    w1: jax.Array,
    b1: jax.Array,
    w2: jax.Array,
    b2: jax.Array,
):
    B, S0, D = x.shape
    S = B * S0
    F = w1.shape[1]

    FM = (F // _LANE) * _LANE
    FT = F - FM
    FP = FM + _LANE
    KH = 256
    FH1 = 768
    FH2 = FP // 2
    assert FT > 0 and 2 * KH <= D and 2 * FH1 <= FM and FP % (2 * _LANE) == 0
    blocks = (512, 256, 768, 512)
    assert sum(blocks) == S
    roff = [int(v) for v in np.concatenate([[0], np.cumsum(blocks)])]
    r0, r1 = blocks[0], blocks[1]
    R01 = r0 + r1
    NPIECE = 4
    pr = r0 // NPIECE
    NPLAIN = 8
    last_rows = (384, 128)
    assert sum(last_rows) == blocks[-1] and NPLAIN % 2 == 0 and NPIECE <= NPLAIN
    queue = ["b1"]
    for i in range(NPLAIN):
        if i < NPIECE:
            queue.append(("x", i * pr, pr))
        queue.append(("w1", i * _LANE, _LANE))
    queue.append(("w1", NPLAIN * _LANE, F - NPLAIN * _LANE))
    n_startup = len(queue)
    queue += [("x", r0, r1), "b2", "w2", ("x", R01, S - R01)]
    SO = len(queue)
    n_out = (len(blocks) - 2) + 1 + len(last_rows) + 1
    PC = 32

    def kernel(x_hbm, w1t_hbm, b1_hbm, w2_hbm, b2_hbm, o_hbm,
               xb, w1b, w2b, b1b, b2b, ob, hb, b1c, tb, ub, sem, order_sem):
        copy = pltpu.make_async_copy
        loads = {}
        for i, q in enumerate(queue):
            if q == "b1":
                loads[q] = copy(b1_hbm, b1b, sem.at[i])
            elif q == "b2":
                loads[q] = copy(b2_hbm, b2b, sem.at[i])
            elif q == "w2":
                loads[q] = copy(w2_hbm, w2b.at[pl.ds(0, F)], sem.at[i])
            else:
                src, dst = (x_hbm, xb) if q[0] == "x" else (w1t_hbm, w1b)
                loads[q] = copy(src.at[pl.ds(q[1], q[2])], dst.at[pl.ds(q[1], q[2])], sem.at[i])
        for q in queue:
            loads[q].start()
        w2b[pl.ds(F, FP - F), :] = jnp.zeros((FP - F, D), _BF16)

        def schedule_fence():
            pl.semaphore_signal(order_sem, 1)
            pl.semaphore_wait(order_sem, 1)

        def bias_row(ref, a, n):
            return ref[pl.ds(a, n)].astype(_F32).reshape(1, n)

        def p1_plain(r, n, a, fn):
            raw = _dot_nt(xb[pl.ds(r, n), :], w1b[pl.ds(a, fn), :])
            return _gelu(raw + bias_row(b1b, a, fn))

        def p1_tail(r, n):
            ht = _dot_nt(w1b[pl.ds(FM, FT), :], xb[pl.ds(r, n), :])
            bc = b1c[...]
            if n > _LANE:
                bc = jnp.concatenate([bc] * (n // _LANE), axis=1)
            return _gelu(ht + bc).T

        def lhs_combos(r, n):
            m = n // 2
            ra, rb = r, r + m
            X11 = xb[pl.ds(ra, m), 0:KH]
            X12 = xb[pl.ds(ra, m), KH:2 * KH]
            X21 = xb[pl.ds(rb, m), 0:KH]
            X22 = xb[pl.ds(rb, m), KH:2 * KH]
            a11, a12, a21, a22 = [v.astype(_F32) for v in (X11, X12, X21, X22)]
            return ((a11 - a22).astype(_BF16), (a21 - a22).astype(_BF16), X11, X22,
                    (a12 - a11).astype(_BF16), (a21 - a11).astype(_BF16),
                    (a12 - a22).astype(_BF16),
                    xb[pl.ds(ra, m), 2 * KH:D], xb[pl.ds(rb, m), 2 * KH:D])

        def p1_pair(lhs, j):
            S1, S2, S3, S4, S5, S6, S7, x3a, x3b = lhs
            ca = pl.ds(2 * j * _LANE, _LANE)
            cb = pl.ds((2 * j + 1) * _LANE, _LANE)
            tj = pl.ds(j * _LANE, _LANE)
            ba = bias_row(b1b, 2 * j * _LANE, _LANE)
            bb = bias_row(b1b, (2 * j + 1) * _LANE, _LANE)
            w31 = w1b[ca, 2 * KH:D]
            w32 = w1b[cb, 2 * KH:D]
            M3 = _dot_nt(S3, tb[1, tj, :])
            M5 = _dot_nt(S5, w1b[cb, KH:2 * KH])
            q12 = _gelu(M3 + M5 + _dot_nt(x3a, w32) + bb)
            M2 = _dot_nt(S2, w1b[ca, 0:KH])
            M4 = _dot_nt(S4, tb[2, tj, :])
            q21 = _gelu(M2 + M4 + _dot_nt(x3b, w31) + ba)
            M1 = _dot_nt(S1, tb[0, tj, :])
            M7 = _dot_nt(S7, tb[4, tj, :])
            q11 = _gelu(M1 + M4 - M5 + M7 + _dot_nt(x3a, w31) + ba)
            M6 = _dot_nt(S6, tb[3, tj, :])
            q22 = _gelu(M1 - M2 + M3 + M6 + _dot_nt(x3b, w32) + bb)
            return q11, q12, q21, q22

        def phase1(r, n):
            lhs = lhs_combos(r, n)
            top, bot = [], []
            for j in range(FH1 // _LANE):
                q11, q12, q21, q22 = p1_pair(lhs, j)
                top += [q11, q12]
                bot += [q21, q22]
            main = jnp.concatenate(
                [jnp.concatenate(top, axis=1), jnp.concatenate(bot, axis=1)], axis=0)
            return jnp.concatenate(
                [main, p1_plain(r, n, 2 * FH1, FM - 2 * FH1), p1_tail(r, n)], axis=1)

        def combine_w1():
            for j in range(FH1 // _LANE):
                for q in range(0, _LANE, PC):
                    d = pl.ds(2 * j * _LANE + q, PC)
                    e = pl.ds((2 * j + 1) * _LANE + q, PC)
                    t = pl.ds(j * _LANE + q, PC)
                    B11 = w1b[d, 0:KH].astype(_F32)
                    B12 = w1b[e, 0:KH].astype(_F32)
                    B21 = w1b[d, KH:2 * KH].astype(_F32)
                    B22 = w1b[e, KH:2 * KH].astype(_F32)
                    tb[0, t, :] = (B11 - B22).astype(_BF16)
                    tb[1, t, :] = (B12 + B22).astype(_BF16)
                    tb[2, t, :] = (B21 + B11).astype(_BF16)
                    tb[3, t, :] = (B11 + B12).astype(_BF16)
                    tb[4, t, :] = (B21 + B22).astype(_BF16)

        def combine_w2():
            for a in range(0, FH2, PC):
                d = pl.ds(a, PC)
                e = pl.ds(FH2 + a, PC)
                B11 = w2b[d, 0:KH].astype(_F32)
                B12 = w2b[d, KH:2 * KH].astype(_F32)
                B21 = w2b[e, 0:KH].astype(_F32)
                B22 = w2b[e, KH:2 * KH].astype(_F32)
                ub[0, d, :] = (B11 - B22).astype(_BF16)
                ub[1, d, :] = (B12 + B22).astype(_BF16)
                ub[2, d, :] = (B21 + B11).astype(_BF16)
                ub[3, d, :] = (B11 + B12).astype(_BF16)
                ub[4, d, :] = (B21 + B22).astype(_BF16)

        def p2_plain(G, r, n, c, cn):
            acc = _dot_nn(G.astype(_BF16), w2b[0:F, pl.ds(c, cn)])
            ob[pl.ds(r, n), pl.ds(c, cn)] = (acc + bias_row(b2b, c, cn)).astype(_BF16)

        def p2_strassen(G, r, n):
            m = n // 2
            Gp = jnp.concatenate([G, jnp.zeros((n, FP - F), _F32)], axis=1)
            G11, G12 = Gp[0:m, 0:FH2], Gp[0:m, FH2:FP]
            G21, G22 = Gp[m:n, 0:FH2], Gp[m:n, FH2:FP]
            ca, cb = pl.ds(0, KH), pl.ds(KH, KH)
            ba, bb = bias_row(b2b, 0, KH), bias_row(b2b, KH, KH)
            P5 = _dot_nn((G12 - G11).astype(_BF16), w2b[FH2:FP, cb])
            P3 = _dot_nn(G11.astype(_BF16), ub[1])
            ob[pl.ds(r, m), cb] = (P3 + P5 + bb).astype(_BF16)
            P2 = _dot_nn((G21 - G22).astype(_BF16), w2b[0:FH2, ca])
            P4 = _dot_nn(G22.astype(_BF16), ub[2])
            ob[pl.ds(r + m, m), ca] = (P2 + P4 + ba).astype(_BF16)
            P1 = _dot_nn((G11 - G22).astype(_BF16), ub[0])
            P7 = _dot_nn((G12 - G22).astype(_BF16), ub[4])
            ob[pl.ds(r, m), ca] = (P1 + P4 - P5 + P7 + ba).astype(_BF16)
            P6 = _dot_nn((G21 - G11).astype(_BF16), ub[3])
            ob[pl.ds(r + m, m), cb] = (P1 - P2 + P3 + P6 + bb).astype(_BF16)

        outs = []

        def write_out(r, n, c, cn):
            if cn == D:
                cp = copy(ob.at[pl.ds(r, n)], o_hbm.at[pl.ds(r, n)], sem.at[SO + len(outs)])
            else:
                cp = copy(ob.at[pl.ds(r, n), pl.ds(c, cn)],
                          o_hbm.at[pl.ds(r, n), pl.ds(c, cn)], sem.at[SO + len(outs)])
            cp.start()
            outs.append(cp)

        loads["b1"].wait()
        bt = bias_row(b1b, FM, FT)
        b1c[...] = jnp.broadcast_to(bt, (_LANE, FT)).T
        x_in, w_in = [], []
        for q in queue[1:n_startup - 1]:
            loads[q].wait()
            if q[0] == "x":
                x_in.append(q)
                todo = [(q, w) for w in w_in]
            else:
                w_in.append(q)
                todo = [(xq, q) for xq in x_in]
            for (_, r, n), (_, a, fn) in todo:
                hb[pl.ds(r, n), pl.ds(a, fn)] = p1_plain(r, n, a, fn)
        loads[queue[n_startup - 1]].wait()
        schedule_fence()
        combine_w1()
        schedule_fence()
        m0 = r0 // 2
        lhs0 = lhs_combos(0, r0)
        for j in range(NPLAIN // 2, FH1 // _LANE):
            q11, q12, q21, q22 = p1_pair(lhs0, j)
            a = 2 * j * _LANE
            hb[pl.ds(0, m0), pl.ds(a, _LANE)] = q11
            hb[pl.ds(0, m0), pl.ds(a + _LANE, _LANE)] = q12
            hb[pl.ds(m0, m0), pl.ds(a, _LANE)] = q21
            hb[pl.ds(m0, m0), pl.ds(a + _LANE, _LANE)] = q22
        hb[pl.ds(0, r0), pl.ds(2 * FH1, FM - 2 * FH1)] = p1_plain(0, r0, 2 * FH1, FM - 2 * FH1)
        hb[pl.ds(0, r0), pl.ds(FM, FT)] = p1_tail(0, r0)

        loads[("x", r0, r1)].wait()
        hb[pl.ds(r0, r1), :] = phase1(r0, r1)
        loads["w2"].wait()
        schedule_fence()
        combine_w2()
        schedule_fence()
        loads["b2"].wait()
        loads[("x", R01, S - R01)].wait()

        G = hb[...]
        p2_strassen(G, 0, R01)
        p2_plain(G, 0, R01, 2 * KH, D - 2 * KH)
        write_out(0, R01, 0, D)

        for i in range(2, len(blocks)):
            r, n = roff[i], blocks[i]
            G = phase1(r, n)
            p2_strassen(G, r, n)
            if i < len(blocks) - 1:
                p2_plain(G, r, n, 2 * KH, D - 2 * KH)
                write_out(r, n, 0, D)
            else:
                write_out(r, n, 0, 2 * KH)
                rr = r
                for rn in last_rows:
                    p2_plain(G[rr - r:rr - r + rn], rr, rn, 2 * KH, D - 2 * KH)
                    write_out(rr, rn, 2 * KH, D - 2 * KH)
                    rr += rn
        for cp in outs:
            cp.wait()

    any_space = pl.BlockSpec(memory_space=pl.ANY)
    out = pl.pallas_call(
        kernel,
        in_specs=[any_space] * 5,
        out_specs=any_space,
        out_shape=jax.ShapeDtypeStruct((S, D), x.dtype),
        scratch_shapes=[
            pltpu.VMEM((S, D), _BF16),
            pltpu.VMEM((F, D), _BF16),
            pltpu.VMEM((FP, D), _BF16),
            pltpu.VMEM((F,), _BF16),
            pltpu.VMEM((D,), _BF16),
            pltpu.VMEM((S, D), _BF16),
            pltpu.VMEM((R01, F), _F32),
            pltpu.VMEM((FT, _LANE), _F32),
            pltpu.VMEM((5, FH1, KH), _BF16),
            pltpu.VMEM((5, FH2, KH), _BF16),
            pltpu.SemaphoreType.DMA((SO + n_out,)),
            pltpu.SemaphoreType.REGULAR,
        ],
        compiler_params=pltpu.CompilerParams(
            vmem_limit_bytes=100 * 1024 * 1024,
            disable_semaphore_checks=True,
            flags={"XLA_TPU_RESCHEDULE_DMA_DONES": True}),
    )(x.reshape(S, D), w1.T, b1, w2, b2)
    return out.reshape(B, S0, D)
```

```python
import jax
import jax.experimental.pallas as pl
import jax.experimental.pallas.tpu as pltpu
import jax.numpy as jnp
import numpy as np
from jax import lax

_F32 = jnp.float32
_BF16 = jnp.bfloat16
_LANE = 128
_NT = (((1,), (1,)), ((), ()))


def _gelu(h):
    c = np.float32(np.sqrt(2.0 / np.pi))
    inner = c * (h + np.float32(0.044715) * (h * h * h))
    return np.float32(0.5) * h * (np.float32(1.0) + jnp.tanh(inner))


def _dot_nt(a, b):
    return lax.dot_general(a, b, _NT, preferred_element_type=_F32)


def _dot_nn(a, b):
    return jnp.dot(a, b, preferred_element_type=_F32)


@jax.jit
def pallas_standalone__dense_activation_gelu__prompt_kernel(
    x: jax.Array,
    w1: jax.Array,
    b1: jax.Array,
    w2: jax.Array,
    b2: jax.Array,
):
    B, S0, D = x.shape
    S = B * S0
    F = w1.shape[1]

    FM = (F // _LANE) * _LANE
    FT = F - FM
    FP = FM + _LANE
    KH = 256
    FH1 = 768
    FH2 = FP // 2
    assert FT > 0 and 2 * KH <= D and 2 * FH1 <= FM and FP % (2 * _LANE) == 0
    blocks = (512, 512, 512, 512)
    assert sum(blocks) == S
    roff = [int(v) for v in np.concatenate([[0], np.cumsum(blocks)])]
    r0, r1 = blocks[0], blocks[1]
    R01 = r0 + r1
    NPIECE = 4
    pr = r0 // NPIECE
    NPLAIN = 8
    last_rows = (256, 128, 128)
    assert sum(last_rows) == blocks[-1] and NPLAIN % 2 == 0 and NPIECE <= NPLAIN
    queue = ["b1"]
    for i in range(NPLAIN):
        if i < NPIECE:
            queue.append(("x", i * pr, pr))
        queue.append(("w1", i * _LANE, _LANE))
    queue.append(("w1", NPLAIN * _LANE, F - NPLAIN * _LANE))
    n_startup = len(queue)
    queue += [("x", r0, r1), "b2", "w2", ("x", R01, S - R01)]
    SO = len(queue)
    n_out = (len(blocks) - 2) + 1 + len(last_rows) + 1
    PC = 32

    def kernel(x_hbm, w1t_hbm, b1_hbm, w2_hbm, b2_hbm, o_hbm,
               xb, w1b, w2b, b1b, b2b, ob, hb, b1c, tb, ub, sem, order_sem):
        copy = pltpu.make_async_copy
        loads = {}
        for i, q in enumerate(queue):
            if q == "b1":
                loads[q] = copy(b1_hbm, b1b, sem.at[i])
            elif q == "b2":
                loads[q] = copy(b2_hbm, b2b, sem.at[i])
            elif q == "w2":
                loads[q] = copy(w2_hbm, w2b.at[pl.ds(0, F)], sem.at[i])
            else:
                src, dst = (x_hbm, xb) if q[0] == "x" else (w1t_hbm, w1b)
                loads[q] = copy(src.at[pl.ds(q[1], q[2])], dst.at[pl.ds(q[1], q[2])], sem.at[i])
        for q in queue:
            loads[q].start()
        w2b[pl.ds(F, FP - F), :] = jnp.zeros((FP - F, D), _BF16)

        def schedule_fence():
            pl.semaphore_signal(order_sem, 1)
            pl.semaphore_wait(order_sem, 1)

        def bias_row(ref, a, n):
            return ref[pl.ds(a, n)].astype(_F32).reshape(1, n)

        def p1_plain(r, n, a, fn):
            raw = _dot_nt(xb[pl.ds(r, n), :], w1b[pl.ds(a, fn), :])
            return _gelu(raw + bias_row(b1b, a, fn))

        def p1_tail(r, n):
            ht = _dot_nt(w1b[pl.ds(FM, FT), :], xb[pl.ds(r, n), :])
            bc = b1c[...]
            if n > _LANE:
                bc = jnp.concatenate([bc] * (n // _LANE), axis=1)
            return _gelu(ht + bc).T

        def lhs_combos(r, n):
            m = n // 2
            ra, rb = r, r + m
            X11 = xb[pl.ds(ra, m), 0:KH]
            X12 = xb[pl.ds(ra, m), KH:2 * KH]
            X21 = xb[pl.ds(rb, m), 0:KH]
            X22 = xb[pl.ds(rb, m), KH:2 * KH]
            a11, a12, a21, a22 = [v.astype(_F32) for v in (X11, X12, X21, X22)]
            return ((a11 - a22).astype(_BF16), (a21 - a22).astype(_BF16), X11, X22,
                    (a12 - a11).astype(_BF16), (a21 - a11).astype(_BF16),
                    (a12 - a22).astype(_BF16),
                    xb[pl.ds(ra, m), 2 * KH:D], xb[pl.ds(rb, m), 2 * KH:D])

        def p1_pair(lhs, j):
            S1, S2, S3, S4, S5, S6, S7, x3a, x3b = lhs
            ca = pl.ds(2 * j * _LANE, _LANE)
            cb = pl.ds((2 * j + 1) * _LANE, _LANE)
            tj = pl.ds(j * _LANE, _LANE)
            ba = bias_row(b1b, 2 * j * _LANE, _LANE)
            bb = bias_row(b1b, (2 * j + 1) * _LANE, _LANE)
            w31 = w1b[ca, 2 * KH:D]
            w32 = w1b[cb, 2 * KH:D]
            M3 = _dot_nt(S3, tb[1, tj, :])
            M5 = _dot_nt(S5, w1b[cb, KH:2 * KH])
            q12 = _gelu(M3 + M5 + _dot_nt(x3a, w32) + bb)
            M2 = _dot_nt(S2, w1b[ca, 0:KH])
            M4 = _dot_nt(S4, tb[2, tj, :])
            q21 = _gelu(M2 + M4 + _dot_nt(x3b, w31) + ba)
            M1 = _dot_nt(S1, tb[0, tj, :])
            M7 = _dot_nt(S7, tb[4, tj, :])
            q11 = _gelu(M1 + M4 - M5 + M7 + _dot_nt(x3a, w31) + ba)
            M6 = _dot_nt(S6, tb[3, tj, :])
            q22 = _gelu(M1 - M2 + M3 + M6 + _dot_nt(x3b, w32) + bb)
            return q11, q12, q21, q22

        def phase1(r, n):
            lhs = lhs_combos(r, n)
            top, bot = [], []
            for j in range(FH1 // _LANE):
                q11, q12, q21, q22 = p1_pair(lhs, j)
                top += [q11, q12]
                bot += [q21, q22]
            main = jnp.concatenate(
                [jnp.concatenate(top, axis=1), jnp.concatenate(bot, axis=1)], axis=0)
            return jnp.concatenate(
                [main, p1_plain(r, n, 2 * FH1, FM - 2 * FH1), p1_tail(r, n)], axis=1)

        def combine_w1():
            for j in range(FH1 // _LANE):
                for q in range(0, _LANE, PC):
                    d = pl.ds(2 * j * _LANE + q, PC)
                    e = pl.ds((2 * j + 1) * _LANE + q, PC)
                    t = pl.ds(j * _LANE + q, PC)
                    B11 = w1b[d, 0:KH].astype(_F32)
                    B12 = w1b[e, 0:KH].astype(_F32)
                    B21 = w1b[d, KH:2 * KH].astype(_F32)
                    B22 = w1b[e, KH:2 * KH].astype(_F32)
                    tb[0, t, :] = (B11 - B22).astype(_BF16)
                    tb[1, t, :] = (B12 + B22).astype(_BF16)
                    tb[2, t, :] = (B21 + B11).astype(_BF16)
                    tb[3, t, :] = (B11 + B12).astype(_BF16)
                    tb[4, t, :] = (B21 + B22).astype(_BF16)

        def combine_w2():
            for a in range(0, FH2, PC):
                d = pl.ds(a, PC)
                e = pl.ds(FH2 + a, PC)
                B11 = w2b[d, 0:KH].astype(_F32)
                B12 = w2b[d, KH:2 * KH].astype(_F32)
                B21 = w2b[e, 0:KH].astype(_F32)
                B22 = w2b[e, KH:2 * KH].astype(_F32)
                ub[0, d, :] = (B11 - B22).astype(_BF16)
                ub[1, d, :] = (B12 + B22).astype(_BF16)
                ub[2, d, :] = (B21 + B11).astype(_BF16)
                ub[3, d, :] = (B11 + B12).astype(_BF16)
                ub[4, d, :] = (B21 + B22).astype(_BF16)

        def p2_plain(G, r, n, c, cn):
            acc = _dot_nn(G.astype(_BF16), w2b[0:F, pl.ds(c, cn)])
            ob[pl.ds(r, n), pl.ds(c, cn)] = (acc + bias_row(b2b, c, cn)).astype(_BF16)

        def p2_strassen(G, r, n):
            m = n // 2
            Gp = jnp.concatenate([G, jnp.zeros((n, FP - F), _F32)], axis=1)
            G11, G12 = Gp[0:m, 0:FH2], Gp[0:m, FH2:FP]
            G21, G22 = Gp[m:n, 0:FH2], Gp[m:n, FH2:FP]
            ca, cb = pl.ds(0, KH), pl.ds(KH, KH)
            ba, bb = bias_row(b2b, 0, KH), bias_row(b2b, KH, KH)
            P5 = _dot_nn((G12 - G11).astype(_BF16), w2b[FH2:FP, cb])
            P3 = _dot_nn(G11.astype(_BF16), ub[1])
            ob[pl.ds(r, m), cb] = (P3 + P5 + bb).astype(_BF16)
            P2 = _dot_nn((G21 - G22).astype(_BF16), w2b[0:FH2, ca])
            P4 = _dot_nn(G22.astype(_BF16), ub[2])
            ob[pl.ds(r + m, m), ca] = (P2 + P4 + ba).astype(_BF16)
            P1 = _dot_nn((G11 - G22).astype(_BF16), ub[0])
            P7 = _dot_nn((G12 - G22).astype(_BF16), ub[4])
            ob[pl.ds(r, m), ca] = (P1 + P4 - P5 + P7 + ba).astype(_BF16)
            P6 = _dot_nn((G21 - G11).astype(_BF16), ub[3])
            ob[pl.ds(r + m, m), cb] = (P1 - P2 + P3 + P6 + bb).astype(_BF16)

        outs = []

        def write_out(r, n, c, cn):
            if cn == D:
                cp = copy(ob.at[pl.ds(r, n)], o_hbm.at[pl.ds(r, n)], sem.at[SO + len(outs)])
            else:
                cp = copy(ob.at[pl.ds(r, n), pl.ds(c, cn)],
                          o_hbm.at[pl.ds(r, n), pl.ds(c, cn)], sem.at[SO + len(outs)])
            cp.start()
            outs.append(cp)

        loads["b1"].wait()
        bt = bias_row(b1b, FM, FT)
        b1c[...] = jnp.broadcast_to(bt, (_LANE, FT)).T
        x_in, w_in = [], []
        for q in queue[1:n_startup - 1]:
            loads[q].wait()
            if q[0] == "x":
                x_in.append(q)
                todo = [(q, w) for w in w_in]
            else:
                w_in.append(q)
                todo = [(xq, q) for xq in x_in]
            for (_, r, n), (_, a, fn) in todo:
                hb[pl.ds(r, n), pl.ds(a, fn)] = p1_plain(r, n, a, fn)
        loads[queue[n_startup - 1]].wait()
        combine_w1()
        schedule_fence()
        m0 = r0 // 2
        lhs0 = lhs_combos(0, r0)
        for j in range(NPLAIN // 2, FH1 // _LANE):
            q11, q12, q21, q22 = p1_pair(lhs0, j)
            a = 2 * j * _LANE
            hb[pl.ds(0, m0), pl.ds(a, _LANE)] = q11
            hb[pl.ds(0, m0), pl.ds(a + _LANE, _LANE)] = q12
            hb[pl.ds(m0, m0), pl.ds(a, _LANE)] = q21
            hb[pl.ds(m0, m0), pl.ds(a + _LANE, _LANE)] = q22
        hb[pl.ds(0, r0), pl.ds(2 * FH1, FM - 2 * FH1)] = p1_plain(0, r0, 2 * FH1, FM - 2 * FH1)
        hb[pl.ds(0, r0), pl.ds(FM, FT)] = p1_tail(0, r0)

        loads[("x", r0, r1)].wait()
        hb[pl.ds(r0, r1), :] = phase1(r0, r1)
        loads["w2"].wait()
        loads["b2"].wait()

        p2_plain(hb[pl.ds(0, r0), :], 0, r0, 2 * KH, D - 2 * KH)
        combine_w2()
        p2_plain(hb[pl.ds(r0, r1), :], r0, r1, 2 * KH, D - 2 * KH)
        schedule_fence()
        loads[("x", R01, S - R01)].wait()
        p2_strassen(hb[...], 0, R01)
        write_out(0, R01, 0, D)

        for i in range(2, len(blocks)):
            r, n = roff[i], blocks[i]
            G = phase1(r, n)
            p2_strassen(G, r, n)
            if i < len(blocks) - 1:
                p2_plain(G, r, n, 2 * KH, D - 2 * KH)
                write_out(r, n, 0, D)
            else:
                write_out(r, n, 0, 2 * KH)
                rr = r
                for rn in last_rows:
                    p2_plain(G[rr - r:rr - r + rn], rr, rn, 2 * KH, D - 2 * KH)
                    write_out(rr, rn, 2 * KH, D - 2 * KH)
                    rr += rn
        for cp in outs:
            cp.wait()

    any_space = pl.BlockSpec(memory_space=pl.ANY)
    out = pl.pallas_call(
        kernel,
        in_specs=[any_space] * 5,
        out_specs=any_space,
        out_shape=jax.ShapeDtypeStruct((S, D), x.dtype),
        scratch_shapes=[
            pltpu.VMEM((S, D), _BF16),
            pltpu.VMEM((F, D), _BF16),
            pltpu.VMEM((FP, D), _BF16),
            pltpu.VMEM((F,), _BF16),
            pltpu.VMEM((D,), _BF16),
            pltpu.VMEM((S, D), _BF16),
            pltpu.VMEM((R01, F), _F32),
            pltpu.VMEM((FT, _LANE), _F32),
            pltpu.VMEM((5, FH1, KH), _BF16),
            pltpu.VMEM((5, FH2, KH), _BF16),
            pltpu.SemaphoreType.DMA((SO + n_out,)),
            pltpu.SemaphoreType.REGULAR,
        ],
        compiler_params=pltpu.CompilerParams(
            vmem_limit_bytes=100 * 1024 * 1024,
            disable_semaphore_checks=True,
            flags={"XLA_TPU_RESCHEDULE_DMA_DONES": True}),
    )(x.reshape(S, D), w1.T, b1, w2, b2)
    return out.reshape(B, S0, D)
```

```python
import jax
import jax.experimental.pallas as pl
import jax.experimental.pallas.tpu as pltpu
import jax.numpy as jnp
import numpy as np
from jax import lax

_F32 = jnp.float32
_BF16 = jnp.bfloat16
_LANE = 128
_NT = (((1,), (1,)), ((), ()))


def _gelu(h):
    c = np.float32(np.sqrt(2.0 / np.pi))
    inner = c * (h + np.float32(0.044715) * (h * h * h))
    return np.float32(0.5) * h * (np.float32(1.0) + jnp.tanh(inner))


def _dot_nt(a, b):
    return lax.dot_general(a, b, _NT, preferred_element_type=_F32)


def _dot_nn(a, b):
    return jnp.dot(a, b, preferred_element_type=_F32)


@jax.jit
def pallas_standalone__dense_activation_gelu__prompt_kernel(
    x: jax.Array,
    w1: jax.Array,
    b1: jax.Array,
    w2: jax.Array,
    b2: jax.Array,
):
    B, S0, D = x.shape
    S = B * S0
    F = w1.shape[1]

    FM = (F // _LANE) * _LANE
    FT = F - FM
    assert 0 < FT < _LANE
    blocks = (512, 512, 512, 512)
    assert sum(blocks) == S
    roff = [int(v) for v in np.concatenate([[0], np.cumsum(blocks)])]
    r0, r1 = blocks[0], blocks[1]
    R01 = r0 + r1
    NPIECE = 4
    pr = r0 // NPIECE
    CSPLIT = 512
    last_slabs = [(roff[-2], blocks[-1], 0, CSPLIT)]
    rr = roff[-2]
    for rn in (384, 64, 64):
        last_slabs.append((rr, rn, CSPLIT, D - CSPLIT))
        rr += rn
    assert rr == S
    queue = ["b1"]
    for i in range(FM // _LANE):
        queue.append(("w1", i * _LANE, _LANE))
        if i < NPIECE:
            queue.append(("x", i * pr, pr))
    n_startup = len(queue)
    queue += [("w1", FM, FT), ("x", r0, r1), "b2", "w2", ("x", R01, S - R01)]
    SO = len(queue)
    n_out = (len(blocks) - 2) + len(last_slabs)

    def kernel(x_hbm, w1t_hbm, b1_hbm, w2_hbm, b2_hbm, o_hbm,
               xb, w1b, w2b, b1b, b2b, ob, hb, b1c, sem):
        copy = pltpu.make_async_copy
        loads = {}
        for i, q in enumerate(queue):
            if q == "b1":
                loads[q] = copy(b1_hbm, b1b, sem.at[i])
            elif q == "b2":
                loads[q] = copy(b2_hbm, b2b, sem.at[i])
            elif q == "w2":
                loads[q] = copy(w2_hbm, w2b, sem.at[i])
            else:
                src, dst = (x_hbm, xb) if q[0] == "x" else (w1t_hbm, w1b)
                loads[q] = copy(src.at[pl.ds(q[1], q[2])], dst.at[pl.ds(q[1], q[2])], sem.at[i])
        for q in queue:
            loads[q].start()

        def bias_row(ref, a, n):
            return ref[pl.ds(a, n)].astype(_F32).reshape(1, n)

        def hidden(r, n, a, fn):
            raw = _dot_nt(xb[pl.ds(r, n), :], w1b[pl.ds(a, fn), :])
            return _gelu(raw + bias_row(b1b, a, fn)).astype(_BF16)

        def hidden_tail(r, n):
            ht = _dot_nt(w1b[pl.ds(FM, FT), :], xb[pl.ds(r, n), :])
            bc = b1c[...]
            if n > _LANE:
                bc = jnp.concatenate([bc] * (n // _LANE), axis=1)
            return _gelu(ht + bc).T.astype(_BF16)

        def project(h, r, n, c, cn):
            acc = _dot_nn(h, w2b[:, pl.ds(c, cn)])
            ob[pl.ds(r, n), pl.ds(c, cn)] = (acc + bias_row(b2b, c, cn)).astype(_BF16)

        outs = []

        def write_out(r, n, c, cn):
            if cn == D:
                cp = copy(ob.at[pl.ds(r, n)], o_hbm.at[pl.ds(r, n)], sem.at[SO + len(outs)])
            else:
                cp = copy(ob.at[pl.ds(r, n), pl.ds(c, cn)],
                          o_hbm.at[pl.ds(r, n), pl.ds(c, cn)], sem.at[SO + len(outs)])
            cp.start()
            outs.append(cp)

        loads["b1"].wait()
        bt = bias_row(b1b, FM, FT)
        b1c[...] = jnp.broadcast_to(bt, (_LANE, FT)).T
        x_in, w_in = [], []
        for q in queue[1:n_startup]:
            loads[q].wait()
            if q[0] == "x":
                x_in.append(q)
                todo = [(q, w) for w in w_in]
            else:
                w_in.append(q)
                todo = [(xq, q) for xq in x_in]
            for (_, r, n), (_, a, fn) in todo:
                hb[pl.ds(r, n), pl.ds(a, fn)] = hidden(r, n, a, fn)
        loads[("w1", FM, FT)].wait()
        hb[pl.ds(0, r0), pl.ds(FM, FT)] = hidden_tail(0, r0)

        loads[("x", r0, r1)].wait()
        hb[pl.ds(r0, r1), pl.ds(0, FM)] = hidden(r0, r1, 0, FM)
        hb[pl.ds(r0, r1), pl.ds(FM, FT)] = hidden_tail(r0, r1)
        loads["w2"].wait()
        loads["b2"].wait()
        loads[("x", R01, S - R01)].wait()

        project(hb[pl.ds(0, r0), :], 0, r0, 0, D)
        project(hb[pl.ds(r0, r1), :], r0, r1, 0, D)
        write_out(0, R01, 0, D)

        for i in range(2, len(blocks)):
            r, n = roff[i], blocks[i]
            h = jnp.concatenate([hidden(r, n, 0, FM), hidden_tail(r, n)], axis=1)
            if i < len(blocks) - 1:
                project(h, r, n, 0, D)
                write_out(r, n, 0, D)
            else:
                for (sr, sn, sc, scn) in last_slabs:
                    project(h if sn == n else h[sr - r:sr - r + sn], sr, sn, sc, scn)
                    write_out(sr, sn, sc, scn)
        for cp in outs:
            cp.wait()

    any_space = pl.BlockSpec(memory_space=pl.ANY)
    out = pl.pallas_call(
        kernel,
        in_specs=[any_space] * 5,
        out_specs=any_space,
        out_shape=jax.ShapeDtypeStruct((S, D), x.dtype),
        scratch_shapes=[
            pltpu.VMEM((S, D), _BF16),
            pltpu.VMEM((F, D), _BF16),
            pltpu.VMEM((F, D), _BF16),
            pltpu.VMEM((F,), _BF16),
            pltpu.VMEM((D,), _BF16),
            pltpu.VMEM((S, D), _BF16),
            pltpu.VMEM((R01, F), _BF16),
            pltpu.VMEM((FT, _LANE), _F32),
            pltpu.SemaphoreType.DMA((SO + n_out,)),
        ],
        compiler_params=pltpu.CompilerParams(
            vmem_limit_bytes=100 * 1024 * 1024,
            disable_semaphore_checks=True,
            flags={"XLA_TPU_RESCHEDULE_DMA_DONES": True}),
    )(x.reshape(S, D), w1.T, b1, w2, b2)
    return out.reshape(B, S0, D)
```
